```python
import os as _os
_os.environ.setdefault("JAX_PLATFORMS", "cpu")
import jax
import jax.numpy as jnp

def _softmax(x, axis=-1):
    return jax.nn.softmax(x, axis=axis)
def _gelu(x):
    return jax.nn.gelu(x, approximate=True)
def _silu(x):
    return jax.nn.silu(x)
def _sigmoid(x):
    return jax.nn.sigmoid(x)
def _layernorm(x, axis=-1, eps=1e-5):
    m = jnp.mean(x, axis=axis, keepdims=True)
    v = jnp.var(x, axis=axis, keepdims=True)
    return (x - m) / jnp.sqrt(v + eps)
def _scatter_add(tgt, idx, src, axis=0):
    return tgt.at[idx].add(src)
def _segment_sum(src, seg, n):
    return jax.ops.segment_sum(src, seg, n)
class _Rng:
    def __init__(self, key):
        self._k = key
    def _next(self):
        self._k, sub = jax.random.split(self._k)
        return sub
    def normal(self, shape):
        return jax.random.normal(self._next(), shape, dtype=jnp.bfloat16)
    def randint(self, lo, hi, shape):
        return jax.random.randint(self._next(), shape, lo, hi, dtype=jnp.int32)
    def uniform(self, shape, lo=0.0, hi=1.0):
        return jax.random.uniform(self._next(), shape, jnp.bfloat16, lo, hi)
    def permutation(self, n):
        return jax.random.permutation(self._next(), n)


kernel_name = 'parallel_sum__spectral_gfnet__glu_gated_swiglu__prompt'

def setup_inputs():
    _rng = _Rng(jax.random.key(int.from_bytes(__import__("os").urandom(4), "little")))
    _w = (lambda a: (lambda t: t.astype(jnp.bfloat16) if jnp.issubdtype(t.dtype, jnp.floating) else t)(jnp.asarray(a)))
    def _A_setup():
        B, S, D = 1, 2048, 512
        Df = D // 2 + 1
        return {
            "x": _w((lambda *s: _rng.normal(s) * 0.05)(B, S, D)),
            "w_r": _w((lambda *s: _rng.normal(s) * 0.2)(S, Df) * 0.02),
            "w_i": _w((lambda *s: _rng.normal(s) * 0.2)(S, Df) * 0.02),
        }
    _A_in = _A_setup()

    def _B_setup():
        B, S, D, F = 1, 2048, 512, 1376
        return {
            "x": _w((lambda *s: _rng.normal(s) * 0.05)(B, S, D)),
            "w1": _w((lambda *s: _rng.normal(s) * 0.05)(D, F) * (2.0 / D) ** 0.5),
            "w3": _w((lambda *s: _rng.normal(s) * 0.05)(D, F) * (2.0 / D) ** 0.5),
            "w2": _w((lambda *s: _rng.normal(s) * 0.05)(F, D) * (2.0 / F) ** 0.5),
        }
    _B_in = _B_setup()

    return {
        "A_x": _A_in["x"],
        "A_w_r": _A_in["w_r"],
        "A_w_i": _A_in["w_i"],
        "B_x": _B_in["x"],
        "B_w1": _B_in["w1"],
        "B_w3": _B_in["w3"],
        "B_w2": _B_in["w2"],
    }

def reference(A_x, A_w_r, A_w_i, B_x, B_w1, B_w3, B_w2):
    def _A_ref(x, w_r, w_i):
        B, S, D = x.shape
        X = (lambda x, axes=(-2,-1): jnp.fft.rfft2(x.astype(jnp.float32), axes=axes))(x, axes=(-2, -1))
        W = w_r + 1j * w_i
        X = X * W
        y = (lambda x, s, axes=(-2,-1): jnp.fft.irfft2(x, s=s, axes=axes).astype(jnp.bfloat16))(X, (S, D), axes=(-2, -1))
        return y

    def _B_ref(x, w1, w3, w2):
        gate = jnp.einsum("bsd,df->bsf", x, w1)
        up = jnp.einsum("bsd,df->bsf", x, w3)
        h = _silu(gate) * up
        out = jnp.einsum("bsf,fd->bsd", h, w2)
        return out

    x = A_x
    xn = _layernorm(x, axis=-1)
    return x + _A_ref(xn, A_w_r, A_w_i) + _B_ref(xn, B_w1, B_w3, B_w2)
```

```python
import functools
import numpy as np
import ml_dtypes
import jax
import jax.numpy as jnp
from jax import lax
import jax.experimental.pallas as pl
import jax.experimental.pallas.tpu as pltpu

S, D, F = 2048, 512, 1376
NA, NB = 32, 64
BM = 512
BF = ml_dtypes.bfloat16


def _cblock(m):
    return np.block([[m.real, -m.imag], [m.imag, m.real]])


def _consts():
    d = np.arange(D)[:, None]
    c = np.arange(D // 2)[None, :]
    ang = 2 * np.pi * ((d * c) % D) / D
    fd = np.concatenate([np.cos(ang), -np.sin(ang)], 1)
    fd[:, D // 2] = np.cos(np.pi * np.arange(D))
    fi = fd.T * (2.0 / D)
    fi[0] *= 0.5
    fi[D // 2] *= 0.5
    fd = np.concatenate([fd[:256, 0::2], fd[:256, 1::2]], 0)
    fi = np.concatenate([fi[0::2, :256], fi[1::2, :256]], 0)
    k2 = np.arange(NB)[:, None]
    nb = np.arange(NB)[None, :]
    l1 = np.stack([_cblock(np.exp(-2j * np.pi * ((k2 * (a + NA * nb)) % S) / S)) for a in range(NA)])
    l4 = np.stack([_cblock(np.exp(2j * np.pi * ((k2 * (a + NA * nb)) % S) / S).T) for a in range(NA)]) / 64
    a = np.arange(NA)
    f32m = np.exp(-2j * np.pi * ((a[:, None] * a[None, :]) % NA) / NA)
    l2 = np.kron(np.eye(2), _cblock(f32m))
    l3 = np.kron(np.eye(2), _cblock(f32m.conj())) / 32
    f64 = np.exp(-2j * np.pi * ((k2 * nb) % NB) / NB)
    ny = np.zeros((6, 128, 128), np.float64)
    ny[0, :64, :64] = f64.real
    ny[0, 64:, :64] = f64.imag
    tw = np.exp(-2j * np.pi * (k2 * a[None, :]) / S)
    ny[1, :64, :32], ny[1, 64:, :32] = tw.real, tw.imag
    ny[2, :32, :32], ny[3, :32, :32] = f32m.real, f32m.imag
    ny[4, :64, :64], ny[4, :64, 64:] = f64.real / S, f64.imag / S
    return (fd.astype(BF), fi.astype(BF), l1.astype(BF), l4.astype(BF),
            np.stack([l2, l3]).astype(BF), ny.astype(np.float32))


def _mm(a, b):
    return jnp.dot(a, b, preferred_element_type=jnp.float32)


def _nt(a, b):
    return lax.dot_general(a, b, (((1,), (1,)), ((), ())), preferred_element_type=jnp.float32)


def _ld(ref, j, g0, n, w):
    return jnp.concatenate([ref[j, pl.ds((g0 + g) * (w + 1), w), :] for g in range(n)], axis=0)


def _st(ref, j, g0, n, w, v):
    for g in range(n):
        ref[j, pl.ds((g0 + g) * (w + 1), w), :] = v[g * w:(g + 1) * w]


def _kernel(x_h, wr_h, wi_h, w1_h, w3_h, w2_h, fd_h, fi_h, l1_h, l4_h, l23_ref, ny_ref, o_h,
            x_v, wr_v, wi_v, w1_v, w3_v, w2_v, fd_v, fi_v, l1_v, l4_v, o_v,
            xn_s, y_s, wf_s, nyo_s, tmp_s, xsem, wsem, osem):
    bf = jnp.bfloat16
    f32 = jnp.float32
    nblk = S // BM
    xc = [pltpu.make_async_copy(x_h.at[pl.ds(i * BM, BM)], x_v.at[pl.ds(i * BM, BM)], xsem.at[i])
          for i in range(nblk)]
    pairs = [(fd_h, fd_v), (l1_h, l1_v), (wr_h, wr_v), (wi_h, wi_v), (l4_h, l4_v), (fi_h, fi_v),
             (w1_h, w1_v), (w3_h, w3_v), (w2_h, w2_v)]
    wc = [pltpu.make_async_copy(a, b, wsem.at[i]) for i, (a, b) in enumerate(pairs)]
    for c in xc + wc[:2]:
        c.start()

    def ln(i, _):
        r = pl.ds(pl.multiple_of(i * BM, BM), BM)
        pltpu.make_async_copy(x_h.at[r], x_v.at[r], xsem.at[i]).wait()
        x = x_v[r, :].astype(f32)
        m = jnp.mean(x, axis=-1, keepdims=True)
        xc_ = x - m
        v = jnp.mean(xc_ * xc_, axis=-1, keepdims=True)
        xn = xc_ * lax.rsqrt(v + 1e-5)
        for j in range(4):
            _st(xn_s, j, i * 16, 16, 32, xn[:, j * 128:(j + 1) * 128])
        return 0
    lax.fori_loop(0, nblk, ln, 0)

    lane = lax.broadcasted_iota(jnp.int32, (NB, 128), 1)
    for c in wc[2:4]:
        c.start()
    wc[0].wait()
    wc[1].wait()

    def s1(g, bm):
        xs = []
        for t in range(4):
            a = g * 4 + t
            xs.append(jnp.concatenate(
                [xn_s[j, pl.ds(a, NB, stride=NA + 1), :] for j in range(4)], axis=1))
        xa = jnp.concatenate(xs, axis=0)
        ze = _mm((xa[:, :256] + xa[:, 256:]).astype(bf), fd_v[:256, :])
        zo = _mm((xa[:, :256] - xa[:, 256:]).astype(bf), fd_v[256:, :])
        z = jnp.concatenate([ze[:, :128], zo[:, :128], ze[:, 128:], zo[:, 128:]], axis=1)
        for t in range(4):
            a = g * 4 + t
            re = z[t * NB:(t + 1) * NB, :256]
            im = z[t * NB:(t + 1) * NB, 256:]
            bm = jnp.where(lane == a, im[:, 0:1], bm)
            im = jnp.concatenate([jnp.where(lane == 0, 0.0, im[:, :128]), im[:, 128:]], axis=1)
            y = _mm(l1_v[a], jnp.concatenate([re, im], axis=0).astype(bf))
            for p in range(2):
                for j in range(2):
                    y_s[p * 2 + j, pl.ds(a, NB, stride=NA + 1), :] = y[p * NB:(p + 1) * NB, j * 128:(j + 1) * 128]
        return bm
    bm = lax.fori_loop(0, NA // 4, s1, jnp.zeros((NB, 128), f32))

    for c in wc[4:]:
        c.start()
    wc[2].wait()
    wc[3].wait()

    def wcv(i, c):
        out = []
        cols = pl.ds(pl.multiple_of(i * 128, 128), 128)
        for p, ref in enumerate((wr_v, wi_v)):
            tmp_s[p] = ref[:256, cols].astype(f32)
            for j in range(2):
                _st(wf_s, p * 2 + j, i * 2, 2, 64, tmp_s[p, pl.ds(j, 128, stride=2), :].T)
            nr = jnp.broadcast_to(ref[256:257, cols].astype(f32), (128, 128)).T
            out.append(jnp.where(lane == 2 * i, nr[:NB], jnp.where(lane == 2 * i + 1, nr[NB:], c[p])))
        return tuple(out)
    z64 = jnp.zeros((NB, 128), f32)
    wnr, wni = lax.fori_loop(0, NA // 2, wcv, (z64, z64))

    hp = functools.partial(jnp.dot, precision=lax.Precision.HIGHEST, preferred_element_type=f32)
    t = hp(ny_ref[0], jnp.concatenate([bm, z64], axis=0))
    tr, ti = t[:NB], t[NB:]
    cr, ci = ny_ref[1, :NB, :], ny_ref[1, NB:, :]
    ur, ui = tr * cr - ti * ci, tr * ci + ti * cr
    gr, gi = ny_ref[2], ny_ref[3]
    vr, vi = hp(ur, gr) - hp(ui, gi), hp(ur, gi) + hp(ui, gr)
    pr, pi_ = vr * wnr - vi * wni, vr * wni + vi * wnr
    qr, qi = hp(pr, gr) + hp(pi_, gi), hp(pi_, gr) - hp(pr, gi)
    sr, si = qr * cr + qi * ci, qi * cr - qr * ci
    nyo_s[...] = hp(ny_ref[4, :NB, :], jnp.concatenate([sr, si], axis=0))

    def s2(g, _):
        pend = []
        for u in range(4):
            q = g * 4 + u
            yr = jnp.concatenate([_ld(y_s, 0, q * 2, 2, 32), _ld(y_s, 1, q * 2, 2, 32)], axis=1)
            yi = jnp.concatenate([_ld(y_s, 2, q * 2, 2, 32), _ld(y_s, 3, q * 2, 2, 32)], axis=1)
            rhs = jnp.concatenate([yr[:32], yi[:32], yr[32:], yi[32:]], axis=0).astype(bf)
            xx = _mm(l23_ref[0], rhs)
            parts = []
            for h in range(2):
                wq = [wf_s[j, pl.ds(q * 2 + h, NA, stride=NB + 1), :] for j in range(4)]
                wr = jnp.concatenate(wq[:2], axis=1)
                wi = jnp.concatenate(wq[2:], axis=1)
                ar, ai = xx[h * 64:h * 64 + 32], xx[h * 64 + 32:h * 64 + 64]
                parts += [ar * wr - ai * wi, ar * wi + ai * wr]
            o = _mm(l23_ref[1], jnp.concatenate(parts, axis=0).astype(bf))
            orr = jnp.concatenate([o[:32], o[64:96]], axis=0)
            oi = jnp.concatenate([o[32:64], o[96:]], axis=0)
            pend.append((0, q * 2, orr[:, :128]))
            pend.append((1, q * 2, orr[:, 128:]))
            pend.append((2, q * 2, oi[:, :128]))
            pend.append((3, q * 2, oi[:, 128:]))
        for j, g0, v in pend:
            _st(y_s, j, g0, 2, 32, v)
        return 0
    lax.fori_loop(0, NB // 8, s2, 0)

    wc[4].wait()
    wc[5].wait()

    def s4(g, _):
        zs = []
        nyo = nyo_s[...]
        for t in range(4):
            a = g * 4 + t
            v = [y_s[j, pl.ds(a, NB, stride=NA + 1), :] for j in range(4)]
            rhs = jnp.concatenate([jnp.concatenate(v[:2], axis=1), jnp.concatenate(v[2:], axis=1)], axis=0)
            o = _mm(l4_v[a], rhs.astype(bf))
            nq = jnp.sum(jnp.where(lane == a, nyo, 0.0), axis=1, keepdims=True)
            im0 = jnp.where(lane == 0, nq, o[NB:, :128])
            zs.append(jnp.concatenate([o[:NB], im0, o[NB:, 128:]], axis=1))
        za = jnp.concatenate(zs, axis=0)
        ye = _mm(jnp.concatenate([za[:, :128], za[:, 256:384]], axis=1).astype(bf), fi_v[:256, :])
        yo = _mm(jnp.concatenate([za[:, 128:256], za[:, 384:]], axis=1).astype(bf), fi_v[256:, :])
        y = jnp.concatenate([ye + yo, ye - yo], axis=1)
        for t in range(4):
            a = g * 4 + t
            for j in range(4):
                wf_s[j, pl.ds(a, NB, stride=NA + 1), :] = y[t * NB:(t + 1) * NB, j * 128:(j + 1) * 128]
        return 0
    lax.fori_loop(0, NA // 4, s4, 0)

    wc[6].wait()
    wc[7].wait()
    wc[8].wait()

    def glu(i, _):
        r = pl.ds(pl.multiple_of(i * BM, BM), BM)
        xn = jnp.concatenate([_ld(xn_s, j, i * 16, 16, 32) for j in range(4)], axis=1).astype(bf)
        g = _nt(xn, w1_v[...])
        u = _nt(xn, w3_v[...])
        h = (g * jax.nn.sigmoid(g) * u).astype(bf)
        sp = jnp.concatenate([_ld(wf_s, j, i * 16, 16, 32) for j in range(4)], axis=1)
        o_v[r, :] = (x_v[r, :].astype(f32) + sp + _mm(h, w2_v[...])).astype(bf)
        pltpu.make_async_copy(o_v.at[r], o_h.at[r], osem.at[i]).start()
        return 0
    lax.fori_loop(0, nblk, glu, 0)
    for i in range(nblk):
        r = pl.ds(i * BM, BM)
        pltpu.make_async_copy(o_v.at[r], o_h.at[r], osem.at[i]).wait()


@jax.jit
def pallas_parallel_sum__spectral_gfnet__glu_gated_swiglu__prompt_kernel(
    A_x, A_w_r, A_w_i, B_x, B_w1, B_w3, B_w2,
):
    del B_x
    cs = _consts()
    bf = jnp.bfloat16
    big = [A_x.reshape(S, D), A_w_r.T, A_w_i.T, B_w1.T, B_w3.T, B_w2, *cs[:4]]
    out = pl.pallas_call(
        _kernel,
        in_specs=[pl.BlockSpec(memory_space=pltpu.HBM)] * 10 + [pl.BlockSpec(memory_space=pltpu.VMEM)] * 2,
        out_specs=pl.BlockSpec(memory_space=pltpu.HBM),
        out_shape=jax.ShapeDtypeStruct((S, D), bf),
        scratch_shapes=[pltpu.VMEM(a.shape, bf) for a in big] + [
            pltpu.VMEM((S, D), bf),
            pltpu.VMEM((4, S + 64, 128), jnp.float32),
            pltpu.VMEM((4, S + 64, 128), jnp.float32),
            pltpu.VMEM((4, S + 64, 128), jnp.float32),
            pltpu.VMEM((NB, 128), jnp.float32),
            pltpu.VMEM((2, 256, 128), jnp.float32),
            pltpu.SemaphoreType.DMA((S // BM,)),
            pltpu.SemaphoreType.DMA((9,)),
            pltpu.SemaphoreType.DMA((S // BM,)),
        ],
        compiler_params=pltpu.CompilerParams(vmem_limit_bytes=100 * 1024 * 1024),
    )(*big, *cs[4:])
    return out.reshape(A_x.shape)
```
